```python
import jax
import jax.numpy as jnp

def _softmax(x, axis=-1):
    return jax.nn.softmax(x, axis=axis)

def _gelu(x):
    return jax.nn.gelu(x, approximate=True)

def _silu(x):
    return jax.nn.silu(x)

def _sigmoid(x):
    return jax.nn.sigmoid(x)

def _layernorm(x, axis=-1, eps=1e-05):
    m = jnp.mean(x, axis=axis, keepdims=True)
    v = jnp.var(x, axis=axis, keepdims=True)
    return (x - m) / jnp.sqrt(v + eps)

def _scatter_add(tgt, idx, src, axis=0):
    return tgt.at[idx].add(src)

def _segment_sum(src, seg, n):
    return jax.ops.segment_sum(src, seg, n)

class _Rng:

    def __init__(self, key):
        self._k = key

    def _next(self):
        self._k, sub = jax.random.split(self._k)
        return sub

    def normal(self, shape):
        return jax.random.normal(self._next(), shape, dtype=jnp.bfloat16)

    def randint(self, lo, hi, shape):
        return jax.random.randint(self._next(), shape, lo, hi, dtype=jnp.int32)

    def uniform(self, shape, lo=0.0, hi=1.0):
        return jax.random.uniform(self._next(), shape, jnp.bfloat16, lo, hi)

    def permutation(self, n):
        return jax.random.permutation(self._next(), n)
kernel_name = 'adaLN_cond__sliding_block_cached__mixer_s_mlp__decode'

def setup_inputs():
    _rng = _Rng(jax.random.key(int.from_bytes(__import__("os").urandom(4), "little")))
    _w = lambda a: (lambda t: t.astype(jnp.bfloat16) if jnp.issubdtype(t.dtype, jnp.floating) else t)(jnp.asarray(a))

    def _A_setup():
        B, Sq, D = (1, 1, 448)
        Hq, Hkv, Sk, Dh = (16, 8, 65536, 256)
        assert Hq % Hkv == 0, (Hq, Hkv)
        return {'x': _w((lambda *s: _rng.normal(s) * 0.05)(B, Sq, D)), 'k_cache': _w((lambda *s: _rng.normal(s) * 0.05)(B, Hkv, Sk, Dh)), 'v_cache': _w((lambda *s: _rng.normal(s) * 0.05)(B, Hkv, Sk, Dh)), 'wq': _w((lambda *s: _rng.normal(s) * 0.05)(D, Hq * Dh) * D ** (-0.5)), 'wo': _w((lambda *s: _rng.normal(s) * 0.05)(Hq * Dh, D) * (Hq * Dh) ** (-0.5))}
    _A_in = _A_setup()

    def _B_setup():
        B, S, D, F = (1, 1, 448, 1792)
        return {'x': _w((lambda *s: _rng.normal(s) * 0.05)(B, S, D)), 'w1': _w((lambda *s: _rng.normal(s) * 0.05)(D, D) * D ** (-0.5)), 'w2': _w((lambda *s: _rng.normal(s) * 0.05)(D, D) * D ** (-0.5)), 'w3': _w((lambda *s: _rng.normal(s) * 0.05)(D, F) * D ** (-0.5)), 'w4': _w((lambda *s: _rng.normal(s) * 0.05)(F, D) * F ** (-0.5))}
    _B_in = _B_setup()
    return {'A_x': _A_in['x'], 'A_k_cache': _A_in['k_cache'], 'A_v_cache': _A_in['v_cache'], 'A_wq': _A_in['wq'], 'A_wo': _A_in['wo'], 'B_x': _B_in['x'], 'B_w1': _B_in['w1'], 'B_w2': _B_in['w2'], 'B_w3': _B_in['w3'], 'B_w4': _B_in['w4'], 'c': _w((lambda *s: _rng.normal(s) * 0.05)(1, 448)), 'w_mod': _w((lambda *s: _rng.normal(s) * 0.05)(448, 6 * 448) * 448 ** (-0.5))}

def reference(A_x, A_k_cache, A_v_cache, A_wq, A_wo, B_x, B_w1, B_w2, B_w3, B_w4, c, w_mod):

    def _A_ref(x, k_cache, v_cache, wq, wo):
        B, Sq, D = x.shape
        Hq, Dh = (16, 256)
        Hkv, Sk = (k_cache.shape[1], k_cache.shape[2])
        W = min(4096, max(256, Sk // 4))
        rep = Hq // Hkv
        q = (lambda x, *d: x.transpose(*d))((x @ wq).reshape(B, Sq, Hq, Dh), 0, 2, 1, 3)
        k = jnp.repeat(k_cache[:, :, Sk - W:, :], rep, axis=1)
        v = jnp.repeat(v_cache[:, :, Sk - W:, :], rep, axis=1)
        scores = jnp.einsum('bhqd,bhkd->bhqk', q, k) * Dh ** (-0.5)
        p = _softmax(scores, axis=-1)
        o = jnp.einsum('bhqk,bhkd->bhqd', p, v)
        return (lambda x, *d: x.transpose(*d))(o, 0, 2, 1, 3).reshape(B, Sq, Hq * Dh) @ wo

    def _B_ref(x, w1, w2, w3, w4):
        B, S, D = x.shape
        h = _gelu(_layernorm(x, axis=-1) @ w1)
        c = D // 4
        g0 = jnp.pad(h[:, :, 0 * c:1 * c], ((0, 0), (1, 0), (0, 0)))[:, :S, :]
        g1 = jnp.pad(h[:, :, 1 * c:2 * c], ((0, 0), (0, 1), (0, 0)))[:, 1:, :]
        g2 = jnp.pad(h[:, :, 2 * c:3 * c], ((0, 0), (2, 0), (0, 0)))[:, :S, :]
        g3 = jnp.pad(h[:, :, 3 * c:], ((0, 0), (0, 2), (0, 0)))[:, 2:, :]
        hs = jnp.concatenate([g0, g1, g2, g3], axis=-1) @ w2
        x1 = x + hs
        h2 = _gelu(_layernorm(x1, axis=-1) @ w3) @ w4
        return x1 + h2
    x = A_x
    mod = (_silu(c) @ w_mod).reshape(c.shape[0], 6, 1, -1)
    sa, ca, ga, sb, cb, gb = (mod[:, 0].copy(), mod[:, 1].copy(), mod[:, 2].copy(), mod[:, 3].copy(), mod[:, 4].copy(), mod[:, 5].copy())
    h = _layernorm(x, axis=-1) * (1 + ca) + sa
    x = x + ga * _A_ref(h, A_k_cache, A_v_cache, A_wq, A_wo)
    h = _layernorm(x, axis=-1) * (1 + cb) + sb
    x = x + gb * _B_ref(h, B_w1, B_w2, B_w3, B_w4)
    return x
```

```python
import jax
import jax.numpy as jnp
import jax.experimental.pallas as pl
import jax.experimental.pallas.tpu as pltpu

_HQ = 16
_DH = 256
_EPS = 1e-05
_NT = (((1,), (1,)), ((), ()))
_NN = (((1,), (0,)), ((), ()))


def _layernorm(x):
    m = jnp.mean(x, axis=-1, keepdims=True)
    d = x - m
    v = jnp.mean(d * d, axis=-1, keepdims=True)
    return d / jnp.sqrt(v + _EPS)


def _dot(a, b, dims):
    return jax.lax.dot_general(a.astype(jnp.bfloat16), b, dims,
                               preferred_element_type=jnp.float32)


@jax.jit
def pallas_adaLN_cond__sliding_block_cached__mixer_s_mlp__decode_kernel(
    A_x: jax.Array,
    A_k_cache: jax.Array,
    A_v_cache: jax.Array,
    A_wq: jax.Array,
    A_wo: jax.Array,
    B_x: jax.Array,
    B_w1: jax.Array,
    B_w2: jax.Array,
    B_w3: jax.Array,
    B_w4: jax.Array,
    c: jax.Array,
    w_mod: jax.Array,
):
    B, S, D = A_x.shape
    _, hkv, sk, dh = A_k_cache.shape
    assert (B, S) == (1, 1) and dh == _DH
    win = min(4096, max(256, sk // 4))
    rep = _HQ // hkv
    F = B_w3.shape[1]
    f32, bf16 = jnp.float32, jnp.bfloat16

    def kernel(x_hbm, c_hbm, wmod_hbm, wq_hbm, k_hbm, v_hbm, wo_hbm, w3_hbm, w4_hbm,
               o_ref,
               x_v, c_v, wmod_v, wq_v, k_v, v_v, wo_v, w3_v, w4_v, sems):
        copies = [
            pltpu.make_async_copy(c_hbm, c_v, sems.at[0]),
            pltpu.make_async_copy(x_hbm, x_v, sems.at[1]),
            pltpu.make_async_copy(wmod_hbm, wmod_v, sems.at[2]),
            pltpu.make_async_copy(wq_hbm, wq_v, sems.at[3]),
        ]
        for h in range(hkv):
            copies.append(pltpu.make_async_copy(
                k_hbm.at[0, h, pl.ds(sk - win, win), :], k_v.at[h], sems.at[4 + 2 * h]))
            copies.append(pltpu.make_async_copy(
                v_hbm.at[0, h, pl.ds(sk - win, win), :], v_v.at[h], sems.at[5 + 2 * h]))
        n = 4 + 2 * hkv
        copies.append(pltpu.make_async_copy(wo_hbm, wo_v, sems.at[n]))
        copies.append(pltpu.make_async_copy(w3_hbm, w3_v, sems.at[n + 1]))
        copies.append(pltpu.make_async_copy(w4_hbm, w4_v, sems.at[n + 2]))
        for cp in copies:
            cp.start()

        copies[0].wait()
        cc = c_v[...].astype(f32)
        sc = jnp.broadcast_to(cc * jax.nn.sigmoid(cc), (8, D))
        copies[2].wait()
        mod = _dot(sc, wmod_v[...], _NN)
        sa, ca, ga, sb, cb, gb = (mod[:, i * D:(i + 1) * D] for i in range(6))
        copies[1].wait()
        x = jnp.broadcast_to(x_v[0].astype(f32), (8, D))
        h = _layernorm(x) * (1 + ca) + sa
        copies[3].wait()
        q = _dot(h, wq_v[...], _NN)
        row = jax.lax.broadcasted_iota(jnp.int32, (8, dh), 0)
        outs = []
        for g in range(hkv):
            qg = jnp.zeros((8, dh), f32)
            for r in range(rep):
                hq = g * rep + r
                qg = jnp.where(row == r, q[:, hq * dh:(hq + 1) * dh], qg)
            copies[4 + 2 * g].wait()
            s = _dot(qg, k_v[g], _NT) * (dh ** -0.5)
            m = jnp.max(s, axis=-1, keepdims=True)
            p = jnp.exp(s - m)
            l = jnp.sum(p, axis=-1, keepdims=True)
            copies[5 + 2 * g].wait()
            og = _dot(p, v_v[g], _NN) / l
            for r in range(rep):
                outs.append(jnp.broadcast_to(og[r:r + 1, :], (8, dh)))
        o = jnp.concatenate(outs, axis=-1)
        copies[n].wait()
        a = _dot(o, wo_v[...], _NT)
        x1 = x + ga * a
        h2 = _layernorm(x1) * (1 + cb) + sb
        copies[n + 1].wait()
        u = jax.nn.gelu(_dot(_layernorm(h2), w3_v[...], _NN), approximate=True)
        copies[n + 2].wait()
        y = h2 + _dot(u, w4_v[...], _NT)
        res = x1 + gb * y
        o_ref[0] = res[0:1, :].astype(o_ref.dtype)

    hbm = pl.BlockSpec(memory_space=pltpu.HBM)
    return pl.pallas_call(
        kernel,
        out_shape=jax.ShapeDtypeStruct(A_x.shape, A_x.dtype),
        in_specs=[hbm] * 9,
        out_specs=pl.BlockSpec(memory_space=pltpu.VMEM),
        scratch_shapes=[
            pltpu.VMEM(A_x.shape, bf16),
            pltpu.VMEM(c.shape, bf16),
            pltpu.VMEM(w_mod.shape, bf16),
            pltpu.VMEM(A_wq.shape, bf16),
            pltpu.VMEM((hkv, win, dh), bf16),
            pltpu.VMEM((hkv, win, dh), bf16),
            pltpu.VMEM((D, _HQ * dh), bf16),
            pltpu.VMEM(B_w3.shape, bf16),
            pltpu.VMEM((D, F), bf16),
            pltpu.SemaphoreType.DMA((7 + 2 * hkv,)),
        ],
        compiler_params=pltpu.CompilerParams(vmem_limit_bytes=100 * 1024 * 1024),
    )(A_x, c, w_mod, A_wq, A_k_cache, A_v_cache, A_wo.T, B_w3, B_w4.T)
```

```python
import contextlib
import jax
import jax.numpy as jnp
import jax.experimental.pallas as pl
import jax.experimental.pallas.tpu as pltpu

_HQ = 16
_EPS = 1e-05
_NT = (((1,), (1,)), ((), ()))
_NN = (((1,), (0,)), ((), ()))
f32, bf16 = jnp.float32, jnp.bfloat16

def _layernorm(x):
    m = jnp.mean(x, axis=-1, keepdims=True)
    d = x - m
    v = jnp.mean(d * d, axis=-1, keepdims=True)
    return d / jnp.sqrt(v + _EPS)

def _dot(a, b, dims):
    return jax.lax.dot_general(a.astype(bf16), b, dims, preferred_element_type=f32)

def rr(nreg, n):
    per = n // nreg
    return [s * per + i for i in range(per) for s in range(nreg)]

SCHED = "bbbbbbvbvbvbvbbWwbwbww"

def make(scopes=False, nochecks=True, diag=None, t_mod=13, t_q=17, lag=8, lead=32, ebatch=8, w4_tail='rows', w4_order=None,
         sched=SCHED, tail_order=None):
    sc_ = (lambda n: jax.named_scope(n)) if scopes else (lambda n: contextlib.nullcontext())
    def scoped(n, fn):
        def g(*a):
            with sc_(n):
                fn(*a)
        return g
    def f(A_x, A_k_cache, A_v_cache, A_wq, A_wo, B_x, B_w1, B_w2, B_w3, B_w4, c, w_mod):
        B, S, D = A_x.shape
        _, hkv, sk, dh = A_k_cache.shape
        win = min(4096, max(256, sk // 4))
        F = B_w3.shape[1]
        hp = 4
        nph = hkv // hp
        TA = 8
        TK = TA + 32 * nph
        S_C, S_X, S_WMOD, S_WQ, S_K = 0, 1, 2, 3, 4
        S_V = S_K + nph
        S_WO = S_V + nph
        S_W3, S_W4 = S_WO + 1, S_WO + 2

        order = [('wo', rg, h) for h in range(2) for rg in rr(7, 56)]
        w3o = [('w3', rg, None) for rg in rr(7, 56)]
        if w4_order is None:
            w4rg = [r for i in range(16) for r in (i, 16 + i)] + list(range(32, 56))
        else:
            w4rg = w4_order
        if w4_tail == 'rows':
            w4o = [('w4', rg, None) for rg in w4rg]
        else:
            nc = w4_tail
            w4o = [('w4', rg, None) for rg in w4rg if rg < 48]
            w4o += [('w4a', rg, nc) for rg in range(48, 56)] + [('w4b', None, nc)]
        order += (w3o + w4o) if tail_order is None else tail_order(w3o, w4o)
        n = len(order)
        n0 = n // 2
        mid = 2 * (n0 - lead)
        s0 = order[:lead] + order[lead:lead + mid:2]
        s1 = order[lead + 1:lead + mid:2] + order[lead + mid:]
        pairs = [(s1[k], s0[k] if k < len(s0) else None) for k in range(len(s1))]
        batches = [pairs[i:i + ebatch] for i in range(0, len(pairs), ebatch)]

        def kernel(x_hbm, c_hbm, wmod_hbm, wq_hbm, k_hbm, v_hbm, wo_hbm, w3_hbm, w4_hbm, o_ref,
                   x_v, c_v, wmod_v, wq_v, k_v, v_v, wo_v, w3_v, w4_v, mod_s, al_s, q_s, p_s, l_s, o_s, sems):
            def cp(src, dst, idx, sem, prio):
                pltpu.make_async_copy(src.at[idx], dst.at[idx], sems.at[sem]).start(priority=prio)
            def wait(buf, sem):
                pltpu.make_async_copy(buf, buf, sems.at[sem]).wait()
            rows8 = lambda rg: pl.ds(rg * 8 if isinstance(rg, int) else pl.multiple_of(rg * 8, 8), 8)
            full = slice(None)

            def issue_a(t, _):
                for half in range(2):
                    for s in range(7):
                        r = rows8(8 * s + t)
                        cp(wq_hbm, wq_v, (r, pl.ds(half * 2048, 2048)), S_WQ, 1)
                        cp(wmod_hbm, wmod_v, (r, pl.ds(half * 1408, 1280 if half else 1408)), S_WMOD, 0)

            def issue_kv(src, dst, sem0, t):
                ph = t >> 4
                i = t & 15
                for j, (hh, reg) in enumerate((hh, reg) for reg in range(4) for hh in range(hp)):
                    row = pl.multiple_of(reg * (win // 4) + i * 64, 64)
                    pltpu.make_async_copy(
                        src.at[0, hp * ph + hh, pl.ds(sk - win + row, 64), :],
                        dst.at[hp * ph + hh, pl.ds(row, 64), :], sems.at[sem0 + ph]).start(priority=1 - j % 2)

            def issue_static(item, prio):
                if item is None:
                    return
                name, rg, h = item
                if name == 'wo':
                    cp(wo_hbm, wo_v, (rows8(rg), pl.ds(h * 2048, 2048)), S_WO, prio)
                elif name == 'w3':
                    cp(w3_hbm, w3_v, (rows8(rg), full), S_W3, prio)
                elif name == 'w4':
                    cp(w4_hbm, w4_v, (rows8(rg), full), S_W4 + rg // 16, prio)
                elif name == 'w4a':
                    cp(w4_hbm, w4_v, (rows8(rg), pl.ds(0, F - h)), S_W4 + 3, prio)
                else:
                    cp(w4_hbm, w4_v, (pl.ds(384, 64), pl.ds(F - h, h)), S_W4 + 4, prio)

            def issue_batch(b):
                for a1, a0 in b:
                    issue_static(a1, 1)
                    issue_static(a0, 0)

            def xval():
                return jnp.broadcast_to(x_v[0].astype(f32), (8, D))

            def do_mod():
                wait(c_v, S_C)
                wait(wmod_v, S_WMOD)
                cc = c_v[...].astype(f32)
                sc = jnp.broadcast_to(cc * jax.nn.sigmoid(cc), (8, D)).astype(bf16)
                def body(j, _):
                    cols = pl.ds(pl.multiple_of(j * 384, 128), 384)
                    mod_s[:, cols] = _dot(sc, wmod_v[:, cols], _NN)
                jax.lax.fori_loop(0, 6 * D // 384, body, None)
                for i in range(6):
                    al_s[i] = mod_s[:, i * D:(i + 1) * D]

            def do_q():
                wait(x_v, S_X)
                wait(wq_v, S_WQ)
                h = (_layernorm(xval()) * (1 + al_s[1]) + al_s[0]).astype(bf16)
                row = jax.lax.broadcasted_iota(jnp.int32, (8, dh), 0)
                def body(g, _):
                    q = _dot(h, wq_v[:, pl.ds(pl.multiple_of(g * 2 * dh, 128), 2 * dh)], _NN)
                    q_s[g] = jnp.where(row == 0, q[:, :dh], q[:, dh:]).astype(bf16)
                jax.lax.fori_loop(0, hkv, body, None)

            def do_qk(g):
                s = _dot(q_s[g], k_v[g], _NT) * (dh ** -0.5)
                p = jnp.exp(s - jnp.max(s, axis=-1, keepdims=True))
                l_s[g] = jnp.broadcast_to(jnp.sum(p, axis=-1, keepdims=True), (8, 128))
                p_s[g] = p.astype(bf16)

            def do_pv(g):
                pv = _dot(p_s[g], v_v[g], _NN)
                o = pv / jnp.concatenate([l_s[g]] * (dh // 128), axis=-1)
                o_s[g] = o.astype(bf16)

            wait_k = lambda ph: wait(k_v.at[pl.ds(hp * ph, hp)], S_K + ph)
            wait_v = lambda ph: wait(v_v.at[pl.ds(hp * ph, hp)], S_V + ph)

            pltpu.make_async_copy(c_hbm, c_v, sems.at[S_C]).start()
            pltpu.make_async_copy(x_hbm, x_v, sems.at[S_X]).start()
            jax.lax.fori_loop(0, TA, issue_a, None)

            def k_step(t, _):
                issue_kv(k_hbm, k_v, S_K, t)
                if diag == 'dma':
                    return
                pl.when(t == t_mod - TA)(scoped('mod', do_mod))
                pl.when(t == t_q - TA)(scoped('q', do_q))
                z = t - 16 - lag
                @pl.when((z >= 0) & ((z & 1) == 0))
                def _():
                    pl.when(z == 0)(lambda: wait_k(0))
                    scoped('qk', do_qk)(z >> 1)
            jax.lax.fori_loop(0, 16 * nph, k_step, None)

            def v_step(t, _):
                issue_kv(v_hbm, v_v, S_V, t)
                if diag == 'dma':
                    return
                z = t - lag
                @pl.when((z >= 0) & (z < 2 * hp) & ((z & 1) == 0))
                def _():
                    pl.when(z == 0)(lambda: wait_k(1))
                    scoped('qk', do_qk)(hp + (z >> 1))
                z2 = t - 16 - lag
                @pl.when((z2 >= 0) & (z2 < hp))
                def _():
                    pl.when(z2 == 0)(lambda: wait_v(0))
                    scoped('pv', do_pv)(z2)
            jax.lax.fori_loop(0, 16 * nph, v_step, None)

            w4_tiles = [(n0, min(128, D - n0)) for n0 in range(0, D, 128)]
            if diag == 'dma':
                for b in batches: issue_batch(b)
                wait(c_v, S_C); wait(x_v, S_X); wait(wmod_v, S_WMOD); wait(wq_v, S_WQ)
                for ph in range(nph):
                    wait_k(ph); wait_v(ph)
                wait(wo_v, S_WO); wait(w3_v, S_W3)
                o_ref[...] = jnp.zeros(o_ref.shape, o_ref.dtype)
                for i, (n0, n) in enumerate(w4_tiles):
                    if i < 3 or w4_tail == 'rows': wait(w4_v.at[pl.ds(n0, n), :], S_W4 + i)
                    else:
                        wait(w4_v.at[pl.ds(n0, n), pl.ds(0, F - w4_tail)], S_W4 + 3)
                        wait(w4_v.at[pl.ds(n0, n), pl.ds(F - w4_tail, w4_tail)], S_W4 + 4)
                return

            ib, iv, iw = 0, hp, 0
            nw = sched.count('w')
            a0 = a1 = jnp.zeros((8, D), f32)
            waited_wo = False
            for ch in sched:
                if ch == 'b':
                    if ib < len(batches):
                        scoped('ebatch', issue_batch)(batches[ib]); ib += 1
                elif ch == 'v':
                    if iv == hp:
                        with sc_('wait_v'): wait_v(1)
                    scoped('pv', do_pv)(iv); iv += 1
                elif ch == 'W':
                    with sc_('wait_wo'): wait(wo_v, S_WO)
                elif ch == 'w':
                    assert iv == hkv
                    with sc_('wo'):
                        for g in range(iw * hkv // nw, (iw + 1) * hkv // nw):
                            og = o_s[g]
                            a0 = a0 + _dot(og, wo_v[:, pl.ds(g * 2 * dh, dh)], _NT)
                            a1 = a1 + _dot(og, wo_v[:, pl.ds(g * 2 * dh + dh, dh)], _NT)
                    iw += 1
            while ib < len(batches):
                scoped('ebatch', issue_batch)(batches[ib]); ib += 1
            with sc_('ln'):
                a = jnp.broadcast_to(a0[0:1] + a1[1:2], (8, D))
                x1 = xval() + al_s[2] * a
                h2 = _layernorm(x1) * (1 + al_s[4]) + al_s[3]
                gb = al_s[5]
                base = x1 + gb * h2
                n2 = _layernorm(h2).astype(bf16)
            with sc_('wait_w3'):
                wait(w3_v, S_W3)
            with sc_('w3'):
                u = jax.nn.gelu(_dot(n2, w3_v[...], _NN), approximate=True).astype(bf16)
            for i, (n0, n) in enumerate(w4_tiles):
                if i < 3 or w4_tail == 'rows':
                    with sc_(f'wait_w4_{i}'):
                        wait(w4_v.at[pl.ds(n0, n), :], S_W4 + i)
                    y = _dot(u, w4_v[pl.ds(n0, n), :], _NT)
                else:
                    nc = w4_tail
                    with sc_(f'wait_w4_{i}a'):
                        wait(w4_v.at[pl.ds(n0, n), pl.ds(0, F - nc)], S_W4 + 3)
                    y = _dot(u[:, :F - nc], w4_v[pl.ds(n0, n), pl.ds(0, F - nc)], _NT)
                    with sc_(f'wait_w4_{i}b'):
                        wait(w4_v.at[pl.ds(n0, n), pl.ds(F - nc, nc)], S_W4 + 4)
                    y = y + _dot(u[:, F - nc:], w4_v[pl.ds(n0, n), pl.ds(F - nc, nc)], _NT)
                res = base[:, n0:n0 + n] + gb[:, n0:n0 + n] * y
                o_ref[0, :, pl.ds(n0, n)] = res[0:1, :].astype(o_ref.dtype)

        hbm = pl.BlockSpec(memory_space=pltpu.HBM)
        return pl.pallas_call(
            kernel,
            out_shape=jax.ShapeDtypeStruct(A_x.shape, A_x.dtype),
            in_specs=[hbm] * 9,
            out_specs=pl.BlockSpec(memory_space=pltpu.VMEM),
            scratch_shapes=[
                pltpu.VMEM(A_x.shape, bf16), pltpu.VMEM(c.shape, bf16), pltpu.VMEM(w_mod.shape, bf16),
                pltpu.VMEM(A_wq.shape, bf16), pltpu.VMEM((hkv, win, dh), bf16), pltpu.VMEM((hkv, win, dh), bf16),
                pltpu.VMEM((D, _HQ * dh), bf16), pltpu.VMEM(B_w3.shape, bf16), pltpu.VMEM((D, F), bf16),
                pltpu.VMEM((8, 6 * D), f32), pltpu.VMEM((6, 8, D), f32), pltpu.VMEM((hkv, 8, dh), bf16),
                pltpu.VMEM((hkv, 8, win), bf16), pltpu.VMEM((hkv, 8, 128), f32), pltpu.VMEM((hkv, 8, dh), bf16),
                pltpu.SemaphoreType.DMA((S_W4 + 5,)),
            ],
            compiler_params=pltpu.CompilerParams(vmem_limit_bytes=100 * 1024 * 1024,
                disable_semaphore_checks=nochecks, disable_bounds_checks=nochecks),
        )(A_x, c, w_mod, A_wq, A_k_cache, A_v_cache, A_wo.T, B_w3, B_w4.T)
    return f


_impl = make()


@jax.jit
def pallas_adaLN_cond__sliding_block_cached__mixer_s_mlp__decode_kernel(
        A_x, A_k_cache, A_v_cache, A_wq, A_wo, B_x, B_w1, B_w2, B_w3, B_w4, c, w_mod):
    return _impl(A_x, A_k_cache, A_v_cache, A_wq, A_wo, B_x, B_w1, B_w2, B_w3, B_w4, c, w_mod)
```

```python
import contextlib
import jax
import jax.numpy as jnp
import jax.experimental.pallas as pl
import jax.experimental.pallas.tpu as pltpu

_HQ = 16
_EPS = 1e-05
_NT = (((1,), (1,)), ((), ()))
_NN = (((1,), (0,)), ((), ()))
f32, bf16 = jnp.float32, jnp.bfloat16

def _layernorm(x):
    m = jnp.mean(x, axis=-1, keepdims=True)
    d = x - m
    v = jnp.mean(d * d, axis=-1, keepdims=True)
    return d / jnp.sqrt(v + _EPS)

def _dot(a, b, dims):
    return jax.lax.dot_general(a.astype(bf16), b, dims, preferred_element_type=f32)

def rr(nreg, n):
    per = n // nreg
    return [s * per + i for i in range(per) for s in range(nreg)]

SCHED = "bbbbbbvbvbvbvbvbvbvbvbWw"
SKEW = (52, 48, 3, 36, 56, 39, 12, 32)

def march(items, ns, skew=0):
    per = len(items) // ns
    assert per * ns == len(items)
    return [items[j * per + (i + skew * j) % per] for i in range(per) for j in range(ns)]

def make(scopes=False, nochecks=True, diag=None, t_mod=13, t_q=17, lag=8, lead=32, ebatch=8, w4_tail='rows', w4_order=None,
         sched=SCHED, tail_order=None, skew_k=SKEW, skew_v=SKEW, wo_ns=8, w3_ns=4, a_skew=1):
    sc_ = (lambda n: jax.named_scope(n)) if scopes else (lambda n: contextlib.nullcontext())
    def scoped(n, fn):
        def g(*a):
            with sc_(n):
                fn(*a)
        return g
    def f(A_x, A_k_cache, A_v_cache, A_wq, A_wo, B_x, B_w1, B_w2, B_w3, B_w4, c, w_mod):
        B, S, D = A_x.shape
        _, hkv, sk, dh = A_k_cache.shape
        win = min(4096, max(256, sk // 4))
        F = B_w3.shape[1]
        hp = hkv
        nph = 1
        TA = 8
        nblk = win // 64
        S_C, S_X, S_WMOD, S_WQ, S_K = 0, 1, 2, 3, 4
        S_V = S_K + nph
        S_WO = S_V + hkv
        S_W3, S_W4 = S_WO + 1, S_WO + 2

        order = march([('wo', rg, h) for rg in range(56) for h in range(2)], wo_ns)
        w3o = march([('w3', rg, None) for rg in range(56)], w3_ns)
        if w4_order is None:
            w4rg = [r for i in range(16) for r in (i, 16 + i)] + list(range(32, 56))
        else:
            w4rg = w4_order
        if w4_tail == 'rows':
            w4o = [('w4', rg, None) for rg in w4rg]
        else:
            nc = w4_tail
            w4o = [('w4', rg, None) for rg in w4rg if rg < 48]
            w4o += [('w4a', rg, nc) for rg in range(48, 56)] + [('w4b', None, nc)]
        order += (w3o + w4o) if tail_order is None else tail_order(w3o, w4o)
        n = len(order)
        n0 = n // 2
        mid = 2 * (n0 - lead)
        s0 = order[:lead] + order[lead:lead + mid:2]
        s1 = order[lead + 1:lead + mid:2] + order[lead + mid:]
        pairs = [(s1[k], s0[k] if k < len(s0) else None) for k in range(len(s1))]
        batches = [pairs[i:i + ebatch] for i in range(0, len(pairs), ebatch)]

        def kernel(x_hbm, c_hbm, wmod_hbm, wq_hbm, k_hbm, v_hbm, wo_hbm, w3_hbm, w4_hbm, o_ref,
                   x_v, c_v, wmod_v, wq_v, k_v, v_v, wo_v, w3_v, w4_v, mod_s, al_s, q_s, p_s, l_s, o_s, sems):
            def cp(src, dst, idx, sem, prio):
                pltpu.make_async_copy(src.at[idx], dst.at[idx], sems.at[sem]).start(priority=prio)
            def wait(buf, sem):
                pltpu.make_async_copy(buf, buf, sems.at[sem]).wait()
            rows8 = lambda rg: pl.ds(rg * 8 if isinstance(rg, int) else pl.multiple_of(rg * 8, 8), 8)
            full = slice(None)

            def issue_a(t, _):
                for half in range(2):
                    for s in range(7):
                        cp(wq_hbm, wq_v, (rows8(8 * s + ((t + a_skew * s) & 7)), pl.ds(half * 2048, 2048)), S_WQ, 1)
                        cp(wmod_hbm, wmod_v, (rows8(8 * s + ((t + a_skew * s + 3) & 7)),
                                              pl.ds(half * 1408, 1280 if half else 1408)), S_WMOD, 0)

            def issue_kv(src, dst, sem, skew, t):
                for k in range(2):
                    for h in range(hkv):
                        row = pl.multiple_of(((2 * t + (k + skew[h])) & (nblk - 1)) * 64, 64)
                        pltpu.make_async_copy(
                            src.at[0, h, pl.ds(sk - win + row, 64), :],
                            dst.at[h, pl.ds(row, 64), :], sems.at[sem(h)]).start(priority=1 - h % 2)

            def issue_static(item, prio):
                if item is None:
                    return
                name, rg, h = item
                if name == 'wo':
                    cp(wo_hbm, wo_v, (rows8(rg), pl.ds(h * 2048, 2048)), S_WO, prio)
                elif name == 'w3':
                    cp(w3_hbm, w3_v, (rows8(rg), full), S_W3, prio)
                elif name == 'w4':
                    cp(w4_hbm, w4_v, (rows8(rg), full), S_W4 + rg // 16, prio)
                elif name == 'w4a':
                    cp(w4_hbm, w4_v, (rows8(rg), pl.ds(0, F - h)), S_W4 + 3, prio)
                else:
                    cp(w4_hbm, w4_v, (pl.ds(384, 64), pl.ds(F - h, h)), S_W4 + 4, prio)

            def issue_batch(b):
                for a1, a0 in b:
                    issue_static(a1, 1)
                    issue_static(a0, 0)

            def xval():
                return jnp.broadcast_to(x_v[0].astype(f32), (8, D))

            def do_mod():
                wait(c_v, S_C)
                wait(wmod_v, S_WMOD)
                cc = c_v[...].astype(f32)
                sc = jnp.broadcast_to(cc * jax.nn.sigmoid(cc), (8, D)).astype(bf16)
                def body(j, _):
                    cols = pl.ds(pl.multiple_of(j * 384, 128), 384)
                    mod_s[:, cols] = _dot(sc, wmod_v[:, cols], _NN)
                jax.lax.fori_loop(0, 6 * D // 384, body, None)
                for i in range(6):
                    al_s[i] = mod_s[:, i * D:(i + 1) * D]

            def do_q():
                wait(x_v, S_X)
                wait(wq_v, S_WQ)
                h = (_layernorm(xval()) * (1 + al_s[1]) + al_s[0]).astype(bf16)
                row = jax.lax.broadcasted_iota(jnp.int32, (8, dh), 0)
                def body(g, _):
                    q = _dot(h, wq_v[:, pl.ds(pl.multiple_of(g * 2 * dh, 128), 2 * dh)], _NN)
                    q_s[g] = jnp.where(row == 0, q[:, :dh], q[:, dh:]).astype(bf16)
                jax.lax.fori_loop(0, hkv, body, None)

            def do_qk(g):
                s = _dot(q_s[g], k_v[g], _NT) * (dh ** -0.5)
                p = jnp.exp(s - jnp.max(s, axis=-1, keepdims=True))
                l_s[g] = jnp.broadcast_to(jnp.sum(p, axis=-1, keepdims=True), (8, 128))
                p_s[g] = p.astype(bf16)

            def do_pv(g):
                pv = _dot(p_s[g], v_v[g], _NN)
                o = pv / jnp.concatenate([l_s[g]] * (dh // 128), axis=-1)
                o_s[g] = o.astype(bf16)

            wait_k = lambda ph: wait(k_v.at[pl.ds(hp * ph, hp)], S_K + ph)
            wait_v = lambda g: wait(v_v.at[g], S_V + g)

            pltpu.make_async_copy(c_hbm, c_v, sems.at[S_C]).start()
            pltpu.make_async_copy(x_hbm, x_v, sems.at[S_X]).start()
            jax.lax.fori_loop(0, TA, issue_a, None)

            def k_step(t, _):
                issue_kv(k_hbm, k_v, lambda h: S_K, skew_k, t)
                if diag == 'dma':
                    return
                pl.when(t == t_mod - TA)(scoped('mod', do_mod))
                pl.when(t == t_q - TA)(scoped('q', do_q))
            jax.lax.fori_loop(0, nblk // 2, k_step, None)

            def v_step(t, _):
                issue_kv(v_hbm, v_v, lambda h: S_V + h, skew_v, t)
                if diag == 'dma':
                    return
                z = t - lag
                @pl.when((z >= 0) & (z < 2 * hkv) & ((z & 1) == 0))
                def _():
                    pl.when(z == 0)(lambda: wait_k(0))
                    scoped('qk', do_qk)(z >> 1)
            jax.lax.fori_loop(0, nblk // 2, v_step, None)

            w4_tiles = [(n0, min(128, D - n0)) for n0 in range(0, D, 128)]
            if diag == 'dma':
                for b in batches: issue_batch(b)
                wait(c_v, S_C); wait(x_v, S_X); wait(wmod_v, S_WMOD); wait(wq_v, S_WQ)
                wait_k(0)
                for g in range(hkv): wait_v(g)
                wait(wo_v, S_WO); wait(w3_v, S_W3)
                o_ref[...] = jnp.zeros(o_ref.shape, o_ref.dtype)
                for i, (n0, n) in enumerate(w4_tiles):
                    if i < 3 or w4_tail == 'rows': wait(w4_v.at[pl.ds(n0, n), :], S_W4 + i)
                    else:
                        wait(w4_v.at[pl.ds(n0, n), pl.ds(0, F - w4_tail)], S_W4 + 3)
                        wait(w4_v.at[pl.ds(n0, n), pl.ds(F - w4_tail, w4_tail)], S_W4 + 4)
                return

            ib, iv, iw = 0, 0, 0
            nw = sched.count('w')
            a0 = a1 = jnp.zeros((8, D), f32)
            waited_wo = False
            for ch in sched:
                if ch == 'b':
                    if ib < len(batches):
                        scoped('ebatch', issue_batch)(batches[ib]); ib += 1
                elif ch == 'v':
                    with sc_('wait_v'): wait_v(iv)
                    scoped('pv', do_pv)(iv); iv += 1
                elif ch == 'W':
                    with sc_('wait_wo'): wait(wo_v, S_WO)
                elif ch == 'w':
                    assert iv == hkv
                    with sc_('wo'):
                        for g in range(iw * hkv // nw, (iw + 1) * hkv // nw):
                            og = o_s[g]
                            a0 = a0 + _dot(og, wo_v[:, pl.ds(g * 2 * dh, dh)], _NT)
                            a1 = a1 + _dot(og, wo_v[:, pl.ds(g * 2 * dh + dh, dh)], _NT)
                    iw += 1
            while ib < len(batches):
                scoped('ebatch', issue_batch)(batches[ib]); ib += 1
            with sc_('ln'):
                a = jnp.broadcast_to(a0[0:1] + a1[1:2], (8, D))
                x1 = xval() + al_s[2] * a
                h2 = _layernorm(x1) * (1 + al_s[4]) + al_s[3]
                gb = al_s[5]
                base = x1 + gb * h2
                n2 = _layernorm(h2).astype(bf16)
            with sc_('wait_w3'):
                wait(w3_v, S_W3)
            with sc_('w3'):
                u = jax.nn.gelu(_dot(n2, w3_v[...], _NN), approximate=True).astype(bf16)
            for i, (n0, n) in enumerate(w4_tiles):
                if i < 3 or w4_tail == 'rows':
                    with sc_(f'wait_w4_{i}'):
                        wait(w4_v.at[pl.ds(n0, n), :], S_W4 + i)
                    y = _dot(u, w4_v[pl.ds(n0, n), :], _NT)
                else:
                    nc = w4_tail
                    with sc_(f'wait_w4_{i}a'):
                        wait(w4_v.at[pl.ds(n0, n), pl.ds(0, F - nc)], S_W4 + 3)
                    y = _dot(u[:, :F - nc], w4_v[pl.ds(n0, n), pl.ds(0, F - nc)], _NT)
                    with sc_(f'wait_w4_{i}b'):
                        wait(w4_v.at[pl.ds(n0, n), pl.ds(F - nc, nc)], S_W4 + 4)
                    y = y + _dot(u[:, F - nc:], w4_v[pl.ds(n0, n), pl.ds(F - nc, nc)], _NT)
                res = base[:, n0:n0 + n] + gb[:, n0:n0 + n] * y
                o_ref[0, :, pl.ds(n0, n)] = res[0:1, :].astype(o_ref.dtype)

        hbm = pl.BlockSpec(memory_space=pltpu.HBM)
        return pl.pallas_call(
            kernel,
            out_shape=jax.ShapeDtypeStruct(A_x.shape, A_x.dtype),
            in_specs=[hbm] * 9,
            out_specs=pl.BlockSpec(memory_space=pltpu.VMEM),
            scratch_shapes=[
                pltpu.VMEM(A_x.shape, bf16), pltpu.VMEM(c.shape, bf16), pltpu.VMEM(w_mod.shape, bf16),
                pltpu.VMEM(A_wq.shape, bf16), pltpu.VMEM((hkv, win, dh), bf16), pltpu.VMEM((hkv, win, dh), bf16),
                pltpu.VMEM((D, _HQ * dh), bf16), pltpu.VMEM(B_w3.shape, bf16), pltpu.VMEM((D, F), bf16),
                pltpu.VMEM((8, 6 * D), f32), pltpu.VMEM((6, 8, D), f32), pltpu.VMEM((hkv, 8, dh), bf16),
                pltpu.VMEM((hkv, 8, win), bf16), pltpu.VMEM((hkv, 8, 128), f32), pltpu.VMEM((hkv, 8, dh), bf16),
                pltpu.SemaphoreType.DMA((S_W4 + 5,)),
            ],
            compiler_params=pltpu.CompilerParams(vmem_limit_bytes=100 * 1024 * 1024,
                disable_semaphore_checks=nochecks, disable_bounds_checks=nochecks),
        )(A_x, c, w_mod, A_wq, A_k_cache, A_v_cache, A_wo.T, B_w3, B_w4.T)
    return f


_impl = make()


@jax.jit
def pallas_adaLN_cond__sliding_block_cached__mixer_s_mlp__decode_kernel(
        A_x, A_k_cache, A_v_cache, A_wq, A_wo, B_x, B_w1, B_w2, B_w3, B_w4, c, w_mod):
    return _impl(A_x, A_k_cache, A_v_cache, A_wq, A_wo, B_x, B_w1, B_w2, B_w3, B_w4, c, w_mod)
```

```python
import contextlib
import jax
import jax.numpy as jnp
import jax.experimental.pallas as pl
import jax.experimental.pallas.tpu as pltpu

_HQ = 16
_EPS = 1e-05
_NT = (((1,), (1,)), ((), ()))
_NN = (((1,), (0,)), ((), ()))
f32, bf16 = jnp.float32, jnp.bfloat16

def _layernorm(x):
    m = jnp.mean(x, axis=-1, keepdims=True)
    d = x - m
    v = jnp.mean(d * d, axis=-1, keepdims=True)
    return d / jnp.sqrt(v + _EPS)

def _dot(a, b, dims):
    return jax.lax.dot_general(a.astype(bf16), b, dims, preferred_element_type=f32)

def ds(start, size, align):
    return pl.ds(pl.multiple_of(start, align), size)

def make(scopes=False, nochecks=True, diag=None, t_mod=4, lag=5, skew=9, skew_v=5, kv_unroll=4,
         keys=1024, pv_keys=1024, nz=2, wo_k=1024, w3_n=896, mod_n=384, a_unroll=1):
    sc_ = (lambda n: jax.named_scope(n)) if scopes else (lambda n: contextlib.nullcontext())
    def scoped(n, fn):
        def g(*a):
            with sc_(n):
                fn(*a)
        return g
    def f(A_x, A_k_cache, A_v_cache, A_wq, A_wo, B_x, B_w1, B_w2, B_w3, B_w4, c, w_mod):
        B, S, D = A_x.shape
        _, hkv, sk, dh = A_k_cache.shape
        win = min(4096, max(256, sk // 4))
        F = B_w3.shape[1]
        nblk = win // 64
        half = nblk // 2
        S_C, S_X, S_WMOD, S_WQ, S_K1, S_K2, S_V1, _a, _b, _c, S_WO, S_W3, S_W4 = range(13)

        def kernel(x_hbm, c_hbm, wmod_hbm, wq_hbm, k_hbm, v_hbm, wo_hbm, w3_hbm, w4_hbm, o_ref,
                   x_v, c_v, wmod_v, wq_v, k_v, v_v, wo_v, w3_v, w4_v, mod_s, al_s, q_s, s_s, p_s, l_s, acc_s, o_s, u_s, y_s, sems):
            def cp(src, dst, idx, sem, prio):
                pltpu.make_async_copy(src.at[idx], dst.at[idx], sems.at[sem]).start(priority=prio)
            def wait(buf, sem):
                pltpu.make_async_copy(buf, buf, sems.at[sem]).wait()

            def issue_a(n, _):
                r = ds((14 * 2 * (n & 1) + (n >> 2)) * 8, 8, 8)
                r2 = ds((14 * (2 * (n & 1) + 1) + (n >> 2)) * 8, 8, 8)
                hf = (n >> 1) & 1
                cols = ds(hf * 2048, 2048, 128)
                cp(wq_hbm, wq_v, (r, cols), S_WQ, 1)
                cp(wq_hbm, wq_v, (r2, cols), S_WQ, 0)
                @pl.when(hf == 0)
                def _():
                    cp(wmod_hbm, wmod_v, (r, pl.ds(0, 1280)), S_WMOD, 1)
                    cp(wmod_hbm, wmod_v, (r2, pl.ds(0, 1280)), S_WMOD, 0)
                @pl.when(hf == 1)
                def _():
                    cp(wmod_hbm, wmod_v, (r, pl.ds(1280, 1408)), S_WMOD, 1)
                    cp(wmod_hbm, wmod_v, (r2, pl.ds(1280, 1408)), S_WMOD, 0)

            def issue_kv(src, dst, sem, t, half, skew):
                base = (2 * t) & (nblk - half)
                def body(j, _):
                    for prio in (1, 0):
                        h = 2 * (j & 3) + 1 - prio
                        row = pl.multiple_of((base + ((2 * t + (j >> 2) + skew * h) & (half - 1))) * 64, 64)
                        pltpu.make_async_copy(src.at[0, h, pl.ds(sk - win + row, 64), :],
                                              dst.at[h, pl.ds(row, 64), :], sems.at[sem]).start(priority=prio)
                jax.lax.fori_loop(0, 8, body, None, unroll=kv_unroll)

            def issue_wo(t):
                def body(j, _):
                    for prio in (1, 0):
                        s = 2 * (j & 3) + 1 - prio
                        cp(wo_hbm, wo_v, (ds((7 * s + t) * 8, 8, 8), ds((j >> 2) * 2048, 2048, 128)), S_WO, prio)
                jax.lax.fori_loop(0, 8, body, None)

            def issue_unit(src, dst, unit, sem, both):
                tpr = F // 128
                for b in range(7):
                    t, end = 16 * b, 16 * b + 16
                    while t < end:
                        g, c0 = divmod(t, tpr)
                        n = min(tpr - c0, end - t)
                        cp(src, dst, (ds(unit * 64 + g * 8, 8, 8), pl.ds(c0 * 128, n * 128)), sem, 1 - (b % 2 if both else 0))
                        t += n

            def xval():
                return jnp.broadcast_to(x_v[0].astype(f32), (8, D))

            def do_mod(j):
                @pl.when(j == 0)
                def _():
                    wait(c_v, S_C)
                    wait(wmod_v, S_WMOD)
                cc = c_v[...].astype(f32)
                sc = jnp.broadcast_to(cc * jax.nn.sigmoid(cc), (8, D))
                cols = ds(j * mod_n, mod_n, 128)
                mod_s[:, cols] = _dot(sc, wmod_v[:, cols], _NN)

            def do_h():
                wait(x_v, S_X)
                wait(wq_v, S_WQ)
                for i in range(2, 6):
                    al_s[i] = mod_s[:, i * D:(i + 1) * D]
                al_s[0] = _layernorm(xval()) * (1 + mod_s[:, D:2 * D]) + mod_s[:, :D]

            def do_q(z):
                def body(i, _):
                    j = 2 * z + i
                    q_s[j] = jnp.broadcast_to(_dot(al_s[0], wq_v[:, ds(j * dh, dh, 128)], _NN), (8, dh))
                jax.lax.fori_loop(0, 2, body, None)

            nck = win // keys // 2
            def do_qk(z):
                hf, g, i = z // (hkv * nck), (z // nck) & (hkv - 1), z & (nck - 1)
                @pl.when(z == 0)
                def _():
                    wait(k_v.at[:, pl.ds(0, win // 2), :], S_K1)
                @pl.when(z == hkv * nck)
                def _():
                    wait(k_v.at[:, pl.ds(win // 2, win // 2), :], S_K2)
                row = jax.lax.broadcasted_iota(jnp.int32, (8, dh), 0)
                q = jnp.where(row == 0, q_s[2 * g], q_s[2 * g + 1])
                j = hf * nck + i
                s_s[g, j] = _dot(q, k_v[g, ds(j * keys, keys, keys), :], _NT) * (dh ** -0.5)
                @pl.when(j == 2 * nck - 1)
                def _():
                    s = s_s[g]
                    m = jnp.max(jnp.max(s, axis=0), axis=-1, keepdims=True)
                    p = jnp.exp(s - m)
                    l_s[g] = jnp.broadcast_to(jnp.sum(jnp.sum(p, axis=0), axis=-1, keepdims=True), (8, 128))
                    p = p.astype(bf16)
                    m_ = keys // pv_keys
                    for a in range(2 * nck):
                        for b in range(m_):
                            p_s[g, a * m_ + b] = p[a, :, b * pv_keys:(b + 1) * pv_keys]

            def v_quarter(i): return v_v.at[:, ds(i * (win // 4), win // 4, win // 4), :]
            def do_pv(z):
                j = z >> 2
                pl.when(z & 3 == 0)(lambda: wait(v_quarter(j), S_V1 + j))
                def body(i, _):
                    g = 2 * (z & 3) + i
                    acc_s[g] += _dot(p_s[g, j], v_v[g, ds(j * pv_keys, pv_keys, pv_keys), :], _NN)
                jax.lax.fori_loop(0, 2, body, None)

            pltpu.make_async_copy(c_hbm, c_v, sems.at[S_C]).start()
            pltpu.make_async_copy(x_hbm, x_v, sems.at[S_X]).start()
            jax.lax.fori_loop(0, 56, issue_a, None, unroll=a_unroll)
            acc_s[...] = jnp.zeros(acc_s.shape, f32)

            T_V, T_WO, T_W3, T_W4 = half, 2 * half, 2 * half + 7, 2 * half + 14
            nmod = 6 * D // mod_n
            t_h = t_mod + nmod
            t_qk = half // 2 + lag
            t_pv = t_qk + 2 * hkv * nck
            def step(t, _):
                pl.when(t < T_V)(lambda: issue_kv(k_hbm, k_v, jnp.where(t < half // 2, S_K1, S_K2), t, half, skew))
                pl.when((t >= T_V) & (t < T_WO))(
                    lambda: issue_kv(v_hbm, v_v, S_V1 + (t - T_V) // (half // 4), t - T_V, nblk // 4, skew_v))
                pl.when((t >= T_WO) & (t < T_W3))(lambda: scoped('iwo', issue_wo)(t - T_WO))
                def u3(i): return ((i & 1) << 2) + (i >> 1)
                pl.when(t >= T_W3)(lambda: scoped('iw3', issue_unit)(w3_hbm, w3_v, u3(t - T_W3), S_W3, True))
                if diag == 'dma':
                    return
                pl.when((t >= t_mod) & (t < t_h))(lambda: scoped('mod', do_mod)(t - t_mod))
                pl.when(t == t_h)(scoped('h', do_h))
                pl.when((t > t_h) & (t <= t_h + _HQ // 2))(lambda: scoped('q', do_q)(t - t_h - 1))
                pl.when((t >= t_qk) & (t < t_qk + 2 * hkv * nck))(lambda: scoped('qk', do_qk)(t - t_qk))
                z1 = t - t_pv
                z2 = t - (T_W3 - 1)
                first = (z1 >= 0) & (z1 < 12)
                pl.when(first | ((z2 >= 0) & (z2 < 4)))(lambda: scoped('pv', do_pv)(jnp.where(first, z1, z2 + 12)))
            jax.lax.fori_loop(0, T_W4, step, None)

            def w4_tile(i): return w4_v.at[pl.ds(128 * i, min(128, D - 128 * i)), :]
            def issue_w4(u): issue_unit(w4_hbm, w4_v, u, S_W4 + (u >> 1), True)
            def issue_w4z(u): issue_unit(w4_hbm, w4_v, u, S_W4 + (u >> 1), False)
            if diag == 'dma':
                jax.lax.fori_loop(0, 7 - nz, lambda u, _: issue_w4(u), None)
                if nz: jax.lax.fori_loop(7 - nz, 7, lambda u, _: issue_w4z(u), None)
                wait(c_v, S_C); wait(x_v, S_X); wait(wmod_v, S_WMOD); wait(wq_v, S_WQ)
                wait(k_v.at[:, pl.ds(0, win // 2), :], S_K1); wait(k_v.at[:, pl.ds(win // 2, win // 2), :], S_K2); [wait(v_quarter(i), S_V1 + i) for i in range(4)]
                wait(wo_v, S_WO); wait(w3_v, S_W3)
                o_ref[...] = jnp.zeros(o_ref.shape, o_ref.dtype)
                for i in range(4): wait(w4_tile(i), S_W4 + i)
                return

            for g in range(hkv):
                o = acc_s[g] / jnp.concatenate([l_s[g]] * (dh // 128), axis=-1)
                for r in range(2):
                    c0 = (2 * g + r) * dh
                    o_s[c0 // wo_k, :, c0 % wo_k:c0 % wo_k + dh] = jnp.broadcast_to(o[r:r + 1], (8, dh)).astype(bf16)

            nwo = _HQ * dh // wo_k
            def wo_step(j, a):
                pl.when(j == 0)(lambda: wait(wo_v, S_WO))
                with sc_('wo'):
                    a = a + _dot(o_s[j], wo_v[:, ds(j * wo_k, wo_k, 128)], _NT)
                per = -(-7 // nwo)
                def body(u, _):
                    pl.when(u < 7 - nz)(lambda: scoped('iw4', issue_w4)(u))
                    if nz: pl.when(u >= 7 - nz)(lambda: scoped('iw4z', issue_w4z)(u))
                jax.lax.fori_loop(j * per, jnp.minimum((j + 1) * per, 7), body, None)
                return a
            a = jax.lax.fori_loop(0, nwo, wo_step, jnp.zeros((8, D), f32))
            with sc_('ln'):
                x1 = xval() + al_s[2] * a
                h2 = _layernorm(x1) * (1 + al_s[4]) + al_s[3]
                gb = al_s[5]
                base = x1 + gb * h2
                n2 = _layernorm(h2).astype(bf16)
            with sc_('wait_w3'):
                wait(w3_v, S_W3)
            with sc_('w3'):
                def body(j, _):
                    cols = ds(j * w3_n, w3_n, 128)
                    u_s[:, cols] = _dot(n2, w3_v[:, cols], _NN)
                jax.lax.fori_loop(0, F // w3_n, body, None)
                u = jax.nn.gelu(u_s[...], approximate=True).astype(bf16)
            def body(i, _):
                rows = ds(i * 128, 128, 128)
                with sc_('wait_w4'):
                    wait(w4_v.at[rows, :], S_W4 + i)
                y_s[i] = _dot(u, w4_v[rows, :], _NT)
            jax.lax.fori_loop(0, 3, body, None)
            with sc_('wait_w4_last'):
                wait(w4_tile(3), S_W4 + 3)
            y = jnp.concatenate([y_s[0], y_s[1], y_s[2], _dot(u, w4_tile(3)[...], _NT)], axis=-1)
            o_ref[0] = (base + gb * y)[0:1, :].astype(o_ref.dtype)

        hbm = pl.BlockSpec(memory_space=pltpu.HBM)
        return pl.pallas_call(
            kernel,
            out_shape=jax.ShapeDtypeStruct(A_x.shape, A_x.dtype),
            in_specs=[hbm] * 9,
            out_specs=pl.BlockSpec(memory_space=pltpu.VMEM),
            scratch_shapes=[
                pltpu.VMEM(A_x.shape, bf16), pltpu.VMEM(c.shape, bf16), pltpu.VMEM(w_mod.shape, bf16),
                pltpu.VMEM(A_wq.shape, bf16), pltpu.VMEM((hkv, win, dh), bf16), pltpu.VMEM((hkv, win, dh), bf16),
                pltpu.VMEM((D, _HQ * dh), bf16), pltpu.VMEM(B_w3.shape, bf16), pltpu.VMEM((D, F), bf16),
                pltpu.VMEM((8, 6 * D), f32), pltpu.VMEM((6, 8, D), f32), pltpu.VMEM((_HQ, 8, dh), f32),
                pltpu.VMEM((hkv, win // keys, 8, keys), f32),
                pltpu.VMEM((hkv, win // pv_keys, 8, pv_keys), bf16), pltpu.VMEM((hkv, 8, 128), f32), pltpu.VMEM((hkv, 8, dh), f32),
                pltpu.VMEM((_HQ * dh // wo_k, 8, wo_k), bf16), pltpu.VMEM((8, F), f32), pltpu.VMEM((3, 8, 128), f32),
                pltpu.SemaphoreType.DMA((S_W4 + 4,)),
            ],
            compiler_params=pltpu.CompilerParams(vmem_limit_bytes=100 * 1024 * 1024,
                disable_semaphore_checks=nochecks, disable_bounds_checks=nochecks),
        )(A_x, c, w_mod, A_wq, A_k_cache, A_v_cache, A_wo.T, B_w3, B_w4.T)
    return f


_impl = make(skew=5, skew_v=3)


@jax.jit
def pallas_adaLN_cond__sliding_block_cached__mixer_s_mlp__decode_kernel(
        A_x, A_k_cache, A_v_cache, A_wq, A_wo, B_x, B_w1, B_w2, B_w3, B_w4, c, w_mod):
    return _impl(A_x, A_k_cache, A_v_cache, A_wq, A_wo, B_x, B_w1, B_w2, B_w3, B_w4, c, w_mod)
```

```python
import jax
import jax.numpy as jnp
import jax.experimental.pallas as pl
import jax.experimental.pallas.tpu as pltpu

_HQ = 16
_EPS = 1e-05
_NN = (((1,), (0,)), ((), ()))
_NT = (((1,), (1,)), ((), ()))
_F32, _BF16 = jnp.float32, jnp.bfloat16

_S_C, _S_X, _S_WMOD, _S_WQ, _S_WO, _S_W3 = range(6)
_S_K, _S_V, _S_W4 = 6, 8, 12
_NUM_SEMS = 16

_BLOCK = 64
_LAG = 6
_LEAD = 12
_WO_COLS = 2048
_W3_COLS = 896


def _layernorm(x):
    m = jnp.mean(x, axis=-1, keepdims=True)
    d = x - m
    v = jnp.mean(d * d, axis=-1, keepdims=True)
    return d / jnp.sqrt(v + _EPS)


def _dot(a, b, dims):
    return jax.lax.dot_general(a.astype(_BF16), b, dims, preferred_element_type=_F32)


def _ds(start, size, align):
    return pl.ds(pl.multiple_of(start, align), size)


def _loop(lo, hi, fn, unroll=None):
    jax.lax.fori_loop(lo, hi, lambda i, _: fn(i), None, unroll=unroll)


def _kernel(x_hbm, c_hbm, wmod_hbm, wq_hbm, k_hbm, v_hbm, wo_hbm, w3_hbm, w4_hbm, o_ref,
            x_v, c_v, wmod_v, wq_v, k_v, v_v, wo_v, w3_v, w4_v,
            mod_s, al_s, q_s, s_s, p_s, l_s, acc_s, o_s, u_s, y_s, sems):
    hkv, win, dh = k_v.shape
    sk = k_hbm.shape[2]
    d, ff = w3_v.shape
    keys = win // 4
    nblk = win // _BLOCK

    def copy(src, dst, idx, sem, priority):
        pltpu.make_async_copy(src.at[idx], dst.at[idx], sems.at[sem]).start(priority=priority)

    def wait(buf, sem):
        pltpu.make_async_copy(buf, buf, sems.at[sem]).wait()

    def mod_rows(n, i):
        return _ds((14 * (2 * (n & 1) + i) + (n >> 2)) * 8, 8, 8)

    def issue_wq(n, priorities):
        for i, priority in enumerate(priorities):
            copy(wq_hbm, wq_v, (mod_rows(n, i), _ds(((n >> 1) & 1) * 2048, 2048, 128)), _S_WQ, priority)

    def issue_wq_wmod(n):
        def issue_wmod(cols):
            for i, priority in enumerate((1, 0)):
                copy(wmod_hbm, wmod_v, (mod_rows(n, i), cols), _S_WMOD, priority)
        pl.when(n >= _LEAD)(lambda: issue_wq(n, (1, 0)))
        pl.when((n & 2) == 0)(lambda: issue_wmod(pl.ds(0, 1280)))
        pl.when((n & 2) != 0)(lambda: issue_wmod(pl.ds(1280, 6 * d - 1280)))

    def issue_cache(src, dst, sem, t, seg, skew):
        base = (2 * t) & (nblk - seg)

        def pair(j):
            for priority in (1, 0):
                h = 2 * (j & 3) + 1 - priority
                blk = base + ((2 * t + (j >> 2) + skew * h) & (seg - 1))
                row = pl.multiple_of(blk * _BLOCK, _BLOCK)
                pltpu.make_async_copy(src.at[0, h, pl.ds(sk - win + row, _BLOCK), :],
                                      dst.at[h, pl.ds(row, _BLOCK), :], sems.at[sem]).start(priority=priority)
        _loop(0, 8, pair, unroll=2)

    def issue_wo(t):
        def pair(j):
            for priority in (1, 0):
                stream = 2 * (j & 3) + 1 - priority
                copy(wo_hbm, wo_v, (_ds((7 * stream + t) * 8, 8, 8), _ds((j >> 2) * 2048, 2048, 128)),
                     _S_WO, priority)
        _loop(0, 8, pair)

    def issue_unit(src, dst, unit, sem, alternate):
        tiles_per_group = ff // 128
        for run in range(tiles_per_group // 2):
            t, end = 16 * run, 16 * run + 16
            while t < end:
                group, col = divmod(t, tiles_per_group)
                n = min(tiles_per_group - col, end - t)
                copy(src, dst, (_ds(unit * 64 + group * 8, 8, 8), pl.ds(col * 128, n * 128)), sem,
                     1 - run % 2 if alternate else 1)
                t += n

    def issue_w4(u):
        pl.when(u < 5)(lambda: issue_unit(w4_hbm, w4_v, u, _S_W4 + (u >> 1), True))
        pl.when(u >= 5)(lambda: issue_unit(w4_hbm, w4_v, u, _S_W4 + (u >> 1), False))

    def x_rows():
        return jnp.broadcast_to(x_v[0].astype(_F32), (8, d))

    def modulation(j):
        @pl.when(j == 0)
        def _():
            wait(c_v, _S_C)
            wait(wmod_v, _S_WMOD)
        cc = c_v[...].astype(_F32)
        cols = _ds(j * 384, 384, 128)
        mod_s[:, cols] = _dot(jnp.broadcast_to(cc * jax.nn.sigmoid(cc), (8, d)), wmod_v[:, cols], _NN)

    def attention_input():
        wait(x_v, _S_X)
        wait(wq_v, _S_WQ)

        def split(i):
            pair = mod_s[:, _ds(i * 2 * d, 2 * d, 128)]
            al_s[2 * i] = pair[:, :d]
            al_s[2 * i + 1] = pair[:, d:]
        _loop(0, 3, split)
        al_s[0] = _layernorm(x_rows()) * (1 + al_s[1]) + al_s[0]

    def queries(z):
        def head(i):
            j = 2 * z + i
            q_s[j] = jnp.broadcast_to(_dot(al_s[0], wq_v[:, _ds(j * dh, dh, 128)], _NN), (8, dh))
        _loop(0, 2, head)

    def scores(z):
        half, g = z >> 4, (z >> 1) & (hkv - 1)

        @pl.when((z & 15) == 0)
        def _():
            wait(k_v.at[:, _ds(half * (win // 2), win // 2, win // 2), :], _S_K + half)
        row = jax.lax.broadcasted_iota(jnp.int32, (8, dh), 0)
        q = jnp.where(row == 0, q_s[2 * g], q_s[2 * g + 1])
        j = 2 * half + (z & 1)
        s_s[g, j] = _dot(q, k_v[g, _ds(j * keys, keys, keys), :], _NT) * (dh ** -0.5)

        @pl.when(j == 3)
        def _():
            m = jax.lax.fori_loop(1, 4, lambda a, m: jnp.maximum(m, s_s[g, a]), s_s[g, 0])
            m = jnp.max(m, axis=-1, keepdims=True)

            def exp_chunk(a, l):
                p = jnp.exp(s_s[g, a] - m)
                p_s[g, a] = p.astype(_BF16)
                return l + p
            l = jax.lax.fori_loop(0, 4, exp_chunk, jnp.zeros((8, keys), _F32))
            l_s[g] = jnp.broadcast_to(jnp.sum(l, axis=-1, keepdims=True), (8, 128))

    def weighted_values(z):
        j = z >> 2
        chunk = _ds(j * keys, keys, keys)
        pl.when((z & 3) == 0)(lambda: wait(v_v.at[:, chunk, :], _S_V + j))

        def head(i):
            g = 2 * (z & 3) + i
            acc_s[g] += _dot(p_s[g, j], v_v[g, chunk, :], _NN)
        _loop(0, 2, head)

    _loop(0, _LEAD, lambda n: issue_wq(n, (1, 1)))
    _loop(0, 56, issue_wq_wmod)
    pltpu.make_async_copy(c_hbm, c_v, sems.at[_S_C]).start()
    pltpu.make_async_copy(x_hbm, x_v, sems.at[_S_X]).start()
    acc_s[...] = jnp.zeros(acc_s.shape, _F32)

    steps = nblk // 2
    t_wo, t_w3, t_end = 2 * steps, 2 * steps + 7, 2 * steps + 14
    t_h = _LAG + 7
    t_qk = steps // 2 + _LAG
    t_pv = t_qk + 32

    def step(t):
        pl.when(t < steps)(
            lambda: issue_cache(k_hbm, k_v, _S_K + t // (steps // 2), t, nblk // 2, 5))
        pl.when((t >= steps) & (t < t_wo))(
            lambda: issue_cache(v_hbm, v_v, _S_V + (t - steps) // (steps // 4), t - steps, nblk // 4, 3))
        pl.when((t >= t_wo) & (t < t_w3))(lambda: issue_wo(t - t_wo))
        i = t - t_w3
        pl.when(i >= 0)(lambda: issue_unit(w3_hbm, w3_v, ((i & 1) << 2) + (i >> 1), _S_W3, True))

        pl.when((t >= _LAG) & (t < t_h))(lambda: modulation(t - _LAG))
        pl.when(t == t_h)(attention_input)
        pl.when((t > t_h) & (t <= t_h + _HQ // 2))(lambda: queries(t - t_h - 1))
        pl.when((t >= t_qk) & (t < t_pv))(lambda: scores(t - t_qk))
        early, late = t - t_pv, t - (t_w3 - 1)
        is_early = (early >= 0) & (early < 12)
        pl.when(is_early | ((late >= 0) & (late < 4)))(
            lambda: weighted_values(jnp.where(is_early, early, late + 12)))
    _loop(0, t_end, step)

    def normalize(g):
        o = acc_s[g] / jnp.concatenate([l_s[g]] * (dh // 128), axis=-1)
        for r in range(2):
            col = (2 * g + r) * dh
            o_s[col // _WO_COLS, :, _ds(col % _WO_COLS, dh, 128)] = jnp.broadcast_to(o[r:r + 1], (8, dh))
    _loop(0, hkv, normalize)

    def project(j, a):
        pl.when(j == 0)(lambda: wait(wo_v, _S_WO))
        a = a + _dot(o_s[j], wo_v[:, _ds(j * _WO_COLS, _WO_COLS, 128)], _NT)
        _loop(4 * j, jnp.minimum(4 * j + 4, 7), issue_w4)
        return a
    a = jax.lax.fori_loop(0, _HQ * dh // _WO_COLS, project, jnp.zeros((8, d), _F32))

    x1 = x_rows() + al_s[2] * a
    h2 = _layernorm(x1) * (1 + al_s[4]) + al_s[3]
    gb = al_s[5]
    base = x1 + gb * h2
    n2 = _layernorm(h2).astype(_BF16)

    wait(w3_v, _S_W3)

    def hidden(j):
        cols = _ds(j * _W3_COLS, _W3_COLS, 128)
        u_s[:, cols] = jax.nn.gelu(_dot(n2, w3_v[:, cols], _NN), approximate=True)
    _loop(0, ff // _W3_COLS, hidden)
    u = u_s[...].astype(_BF16)

    def out_tile(i):
        rows = _ds(i * 128, 128, 128)
        wait(w4_v.at[rows, :], _S_W4 + i)
        y_s[i] = _dot(u, w4_v[rows, :], _NT)
    _loop(0, 3, out_tile)
    last = pl.ds(384, d - 384)
    wait(w4_v.at[last, :], _S_W4 + 3)
    y = jnp.concatenate([y_s[0], y_s[1], y_s[2], _dot(u, w4_v[last, :], _NT)], axis=-1)
    o_ref[0] = (base + gb * y)[0:1, :].astype(o_ref.dtype)


@jax.jit
def pallas_adaLN_cond__sliding_block_cached__mixer_s_mlp__decode_kernel(
    A_x: jax.Array,
    A_k_cache: jax.Array,
    A_v_cache: jax.Array,
    A_wq: jax.Array,
    A_wo: jax.Array,
    B_x: jax.Array,
    B_w1: jax.Array,
    B_w2: jax.Array,
    B_w3: jax.Array,
    B_w4: jax.Array,
    c: jax.Array,
    w_mod: jax.Array,
):
    batch, seq, d = A_x.shape
    _, hkv, sk, dh = A_k_cache.shape
    ff = B_w3.shape[1]
    win = min(4096, max(256, sk // 4))
    assert (batch, seq, d, ff) == (1, 1, 448, 1792) and (hkv, win, dh) == (8, 4096, 256)
    keys = win // 4

    return pl.pallas_call(
        _kernel,
        out_shape=jax.ShapeDtypeStruct(A_x.shape, A_x.dtype),
        in_specs=[pl.BlockSpec(memory_space=pltpu.HBM)] * 9,
        out_specs=pl.BlockSpec(memory_space=pltpu.VMEM),
        scratch_shapes=[
            pltpu.VMEM(A_x.shape, _BF16),
            pltpu.VMEM(c.shape, _BF16),
            pltpu.VMEM(w_mod.shape, _BF16),
            pltpu.VMEM(A_wq.shape, _BF16),
            pltpu.VMEM((hkv, win, dh), _BF16),
            pltpu.VMEM((hkv, win, dh), _BF16),
            pltpu.VMEM((d, _HQ * dh), _BF16),
            pltpu.VMEM((d, ff), _BF16),
            pltpu.VMEM((d, ff), _BF16),
            pltpu.VMEM((8, 6 * d), _F32),
            pltpu.VMEM((6, 8, d), _F32),
            pltpu.VMEM((_HQ, 8, dh), _F32),
            pltpu.VMEM((hkv, 4, 8, keys), _F32),
            pltpu.VMEM((hkv, 4, 8, keys), _BF16),
            pltpu.VMEM((hkv, 8, 128), _F32),
            pltpu.VMEM((hkv, 8, dh), _F32),
            pltpu.VMEM((_HQ * dh // _WO_COLS, 8, _WO_COLS), _F32),
            pltpu.VMEM((8, ff), _F32),
            pltpu.VMEM((3, 8, 128), _F32),
            pltpu.SemaphoreType.DMA((_NUM_SEMS,)),
        ],
        compiler_params=pltpu.CompilerParams(
            vmem_limit_bytes=100 * 1024 * 1024,
            disable_bounds_checks=True,
            disable_semaphore_checks=True,
        ),
    )(A_x, c, w_mod, A_wq, A_k_cache, A_v_cache, A_wo.T, B_w3, B_w4.T)
```

```python
import jax
import jax.numpy as jnp
import jax.experimental.pallas as pl
import jax.experimental.pallas.tpu as pltpu

_HQ = 16
_EPS = 1e-05
_NN = (((1,), (0,)), ((), ()))
_NT = (((1,), (1,)), ((), ()))
_F32, _BF16 = jnp.float32, jnp.bfloat16

_S_C, _S_X, _S_WMOD, _S_WQ, _S_WO, _S_W3 = range(6)
_S_K, _S_V, _S_W4 = 6, 8, 12
_NUM_SEMS = 16

_BLOCK = 64
_LAG = 6
_LEAD = 12
_WO_COLS = 2048
_W3_COLS = 896


def _layernorm(x):
    m = jnp.mean(x, axis=-1, keepdims=True)
    d = x - m
    v = jnp.mean(d * d, axis=-1, keepdims=True)
    return d / jnp.sqrt(v + _EPS)


def _dot(a, b, dims):
    return jax.lax.dot_general(a.astype(_BF16), b, dims, preferred_element_type=_F32)


def _ds(start, size, align):
    return pl.ds(pl.multiple_of(start, align), size)


def _loop(lo, hi, fn, unroll=None):
    jax.lax.fori_loop(lo, hi, lambda i, _: fn(i), None, unroll=unroll)


def _kernel(x_hbm, c_hbm, wmod_hbm, wq_hbm, k_hbm, v_hbm, wo_hbm, w3_hbm, w4_hbm, o_ref,
            x_v, c_v, wmod_v, wq_v, k_v, v_v, wo_v, w3_v, w4_v,
            mod_s, al_s, q_s, s_s, p_s, l_s, acc_s, o_s, u_s, y_s, sems):
    hkv, win, dh = k_v.shape
    sk = k_hbm.shape[2]
    d, ff = w3_v.shape
    keys = win // 4
    nblk = win // _BLOCK

    def copy(src, dst, idx, sem, priority):
        pltpu.make_async_copy(src.at[idx], dst.at[idx], sems.at[sem]).start(priority=priority)

    def wait(buf, sem):
        pltpu.make_async_copy(buf, buf, sems.at[sem]).wait()

    def mod_rows(n, i):
        return _ds((14 * (2 * (n & 1) + i) + (n >> 2)) * 8, 8, 8)

    def issue_wq(n, priorities):
        for i, priority in enumerate(priorities):
            copy(wq_hbm, wq_v, (mod_rows(n, i), _ds(((n >> 1) & 1) * 2048, 2048, 128)), _S_WQ, priority)

    def issue_wq_wmod(n):
        def issue_wmod(cols):
            for i, priority in enumerate((1, 0)):
                copy(wmod_hbm, wmod_v, (mod_rows(n, i), cols), _S_WMOD, priority)
        pl.when(n >= _LEAD)(lambda: issue_wq(n, (1, 0)))
        pl.when((n & 2) == 0)(lambda: issue_wmod(pl.ds(0, 1280)))
        pl.when((n & 2) != 0)(lambda: issue_wmod(pl.ds(1280, 6 * d - 1280)))

    def issue_cache(src, dst, sem, t, seg, skew):
        base = (2 * t) & (nblk - seg)

        def pair(j):
            for priority in (1, 0):
                h = 2 * (j & 3) + 1 - priority
                blk = base + ((2 * t + (j >> 2) + skew * h) & (seg - 1))
                row = pl.multiple_of(blk * _BLOCK, _BLOCK)
                pltpu.make_async_copy(src.at[0, h, pl.ds(sk - win + row, _BLOCK), :],
                                      dst.at[h, pl.ds(row, _BLOCK), :], sems.at[sem]).start(priority=priority)
        _loop(0, 8, pair, unroll=2)

    def issue_wo(t):
        def pair(j):
            for priority in (1, 0):
                stream = 2 * (j & 3) + 1 - priority
                copy(wo_hbm, wo_v, (_ds((7 * stream + t) * 8, 8, 8), _ds((j >> 2) * 2048, 2048, 128)),
                     _S_WO, priority)
        _loop(0, 8, pair)

    def issue_runs(src, dst, unit_of_run, sem, alternate):
        tiles_per_group = ff // 128
        for run in range(tiles_per_group // 2):
            unit = unit_of_run(run)
            t, end = 16 * run, 16 * run + 16
            while t < end:
                group, col = divmod(t, tiles_per_group)
                n = min(tiles_per_group - col, end - t)
                copy(src, dst, (_ds(unit * 64 + group * 8, 8, 8), pl.ds(col * 128, n * 128)), sem,
                     1 - run % 2 if alternate else 1)
                t += n

    def issue_w3(i):
        first = ((i & 1) << 2) + (i >> 1)

        def unit_of_run(run):
            unit = first + (2 * run) % 7
            return jnp.where(unit >= 7, unit - 7, unit)
        issue_runs(w3_hbm, w3_v, unit_of_run, _S_W3, True)

    def issue_w4(u):
        pl.when(u < 5)(lambda: issue_runs(w4_hbm, w4_v, lambda run: u, _S_W4 + (u >> 1), True))
        pl.when(u >= 5)(lambda: issue_runs(w4_hbm, w4_v, lambda run: u, _S_W4 + (u >> 1), False))

    def x_rows():
        return jnp.broadcast_to(x_v[0].astype(_F32), (8, d))

    def modulation(j):
        @pl.when(j == 0)
        def _():
            wait(c_v, _S_C)
            wait(wmod_v, _S_WMOD)
        cc = c_v[...].astype(_F32)
        cols = _ds(j * 384, 384, 128)
        mod_s[:, cols] = _dot(jnp.broadcast_to(cc * jax.nn.sigmoid(cc), (8, d)), wmod_v[:, cols], _NN)

    def attention_input():
        wait(x_v, _S_X)
        wait(wq_v, _S_WQ)

        def split(i):
            pair = mod_s[:, _ds(i * 2 * d, 2 * d, 128)]
            al_s[2 * i] = pair[:, :d]
            al_s[2 * i + 1] = pair[:, d:]
        _loop(0, 3, split)
        al_s[0] = _layernorm(x_rows()) * (1 + al_s[1]) + al_s[0]

    def queries(z):
        def head(i):
            j = 2 * z + i
            q_s[j] = jnp.broadcast_to(_dot(al_s[0], wq_v[:, _ds(j * dh, dh, 128)], _NN), (8, dh))
        _loop(0, 2, head)

    def scores(z):
        half, g = z >> 4, (z >> 1) & (hkv - 1)

        @pl.when((z & 15) == 0)
        def _():
            wait(k_v.at[:, _ds(half * (win // 2), win // 2, win // 2), :], _S_K + half)
        row = jax.lax.broadcasted_iota(jnp.int32, (8, dh), 0)
        q = jnp.where(row == 0, q_s[2 * g], q_s[2 * g + 1])
        j = 2 * half + (z & 1)
        s_s[g, j] = _dot(q, k_v[g, _ds(j * keys, keys, keys), :], _NT) * (dh ** -0.5)

        @pl.when(j == 3)
        def _():
            m = jax.lax.fori_loop(1, 4, lambda a, m: jnp.maximum(m, s_s[g, a]), s_s[g, 0])
            m = jnp.max(m, axis=-1, keepdims=True)

            def exp_chunk(a, l):
                p = jnp.exp(s_s[g, a] - m)
                p_s[g, a] = p.astype(_BF16)
                return l + p
            l = jax.lax.fori_loop(0, 4, exp_chunk, jnp.zeros((8, keys), _F32))
            l_s[g] = jnp.broadcast_to(jnp.sum(l, axis=-1, keepdims=True), (8, 128))

    def weighted_values(z):
        j = z >> 2
        chunk = _ds(j * keys, keys, keys)
        pl.when((z & 3) == 0)(lambda: wait(v_v.at[:, chunk, :], _S_V + j))

        def head(i):
            g = 2 * (z & 3) + i
            acc_s[g] += _dot(p_s[g, j], v_v[g, chunk, :], _NN)
        _loop(0, 2, head)

    _loop(0, _LEAD, lambda n: issue_wq(n, (1, 1)))
    _loop(0, 56, issue_wq_wmod)
    pltpu.make_async_copy(c_hbm, c_v, sems.at[_S_C]).start()
    pltpu.make_async_copy(x_hbm, x_v, sems.at[_S_X]).start()
    acc_s[...] = jnp.zeros(acc_s.shape, _F32)

    steps = nblk // 2
    t_wo, t_w3, t_end = 2 * steps, 2 * steps + 7, 2 * steps + 14
    t_h = _LAG + 7
    t_qk = steps // 2 + _LAG
    t_pv = t_qk + 32

    def step(t):
        pl.when(t < steps)(
            lambda: issue_cache(k_hbm, k_v, _S_K + t // (steps // 2), t, nblk // 2, 5))
        pl.when((t >= steps) & (t < t_wo))(
            lambda: issue_cache(v_hbm, v_v, _S_V + (t - steps) // (steps // 4), t - steps, nblk // 4, 3))
        pl.when((t >= t_wo) & (t < t_w3))(lambda: issue_wo(t - t_wo))
        pl.when(t >= t_w3)(lambda: issue_w3(t - t_w3))

        pl.when((t >= _LAG) & (t < t_h))(lambda: modulation(t - _LAG))
        pl.when(t == t_h)(attention_input)
        pl.when((t > t_h) & (t <= t_h + _HQ // 2))(lambda: queries(t - t_h - 1))
        pl.when((t >= t_qk) & (t < t_pv))(lambda: scores(t - t_qk))
        early, late = t - t_pv, t - (t_w3 - 1)
        is_early = (early >= 0) & (early < 12)
        pl.when(is_early | ((late >= 0) & (late < 4)))(
            lambda: weighted_values(jnp.where(is_early, early, late + 12)))
    _loop(0, t_end, step)

    def normalize(g):
        o = acc_s[g] / jnp.concatenate([l_s[g]] * (dh // 128), axis=-1)
        for r in range(2):
            col = (2 * g + r) * dh
            o_s[col // _WO_COLS, :, _ds(col % _WO_COLS, dh, 128)] = jnp.broadcast_to(o[r:r + 1], (8, dh))
    _loop(0, hkv, normalize)

    def project(j, a):
        pl.when(j == 0)(lambda: wait(wo_v, _S_WO))
        a = a + _dot(o_s[j], wo_v[:, _ds(j * _WO_COLS, _WO_COLS, 128)], _NT)
        _loop(4 * j, jnp.minimum(4 * j + 4, 7), issue_w4)
        return a
    a = jax.lax.fori_loop(0, _HQ * dh // _WO_COLS, project, jnp.zeros((8, d), _F32))

    x1 = x_rows() + al_s[2] * a
    h2 = _layernorm(x1) * (1 + al_s[4]) + al_s[3]
    gb = al_s[5]
    base = x1 + gb * h2
    n2 = _layernorm(h2).astype(_BF16)

    wait(w3_v, _S_W3)

    def hidden(j):
        cols = _ds(j * _W3_COLS, _W3_COLS, 128)
        u_s[:, cols] = jax.nn.gelu(_dot(n2, w3_v[:, cols], _NN), approximate=True)
    _loop(0, ff // _W3_COLS, hidden)
    u = u_s[...].astype(_BF16)

    def out_tile(i):
        rows = _ds(i * 128, 128, 128)
        wait(w4_v.at[rows, :], _S_W4 + i)
        y_s[i] = _dot(u, w4_v[rows, :], _NT)
    _loop(0, 3, out_tile)
    last = pl.ds(384, d - 384)
    wait(w4_v.at[last, :], _S_W4 + 3)
    y = jnp.concatenate([y_s[0], y_s[1], y_s[2], _dot(u, w4_v[last, :], _NT)], axis=-1)
    o_ref[0] = (base + gb * y)[0:1, :].astype(o_ref.dtype)


@jax.jit
def pallas_adaLN_cond__sliding_block_cached__mixer_s_mlp__decode_kernel(
    A_x: jax.Array,
    A_k_cache: jax.Array,
    A_v_cache: jax.Array,
    A_wq: jax.Array,
    A_wo: jax.Array,
    B_x: jax.Array,
    B_w1: jax.Array,
    B_w2: jax.Array,
    B_w3: jax.Array,
    B_w4: jax.Array,
    c: jax.Array,
    w_mod: jax.Array,
):
    batch, seq, d = A_x.shape
    _, hkv, sk, dh = A_k_cache.shape
    ff = B_w3.shape[1]
    win = min(4096, max(256, sk // 4))
    assert (batch, seq, d, ff) == (1, 1, 448, 1792) and (hkv, win, dh) == (8, 4096, 256)
    keys = win // 4

    return pl.pallas_call(
        _kernel,
        out_shape=jax.ShapeDtypeStruct(A_x.shape, A_x.dtype),
        in_specs=[pl.BlockSpec(memory_space=pltpu.HBM)] * 9,
        out_specs=pl.BlockSpec(memory_space=pltpu.VMEM),
        scratch_shapes=[
            pltpu.VMEM(A_x.shape, _BF16),
            pltpu.VMEM(c.shape, _BF16),
            pltpu.VMEM(w_mod.shape, _BF16),
            pltpu.VMEM(A_wq.shape, _BF16),
            pltpu.VMEM((hkv, win, dh), _BF16),
            pltpu.VMEM((hkv, win, dh), _BF16),
            pltpu.VMEM((d, _HQ * dh), _BF16),
            pltpu.VMEM((d, ff), _BF16),
            pltpu.VMEM((d, ff), _BF16),
            pltpu.VMEM((8, 6 * d), _F32),
            pltpu.VMEM((6, 8, d), _F32),
            pltpu.VMEM((_HQ, 8, dh), _F32),
            pltpu.VMEM((hkv, 4, 8, keys), _F32),
            pltpu.VMEM((hkv, 4, 8, keys), _BF16),
            pltpu.VMEM((hkv, 8, 128), _F32),
            pltpu.VMEM((hkv, 8, dh), _F32),
            pltpu.VMEM((_HQ * dh // _WO_COLS, 8, _WO_COLS), _F32),
            pltpu.VMEM((8, ff), _F32),
            pltpu.VMEM((3, 8, 128), _F32),
            pltpu.SemaphoreType.DMA((_NUM_SEMS,)),
        ],
        compiler_params=pltpu.CompilerParams(
            vmem_limit_bytes=100 * 1024 * 1024,
            disable_bounds_checks=True,
            disable_semaphore_checks=True,
        ),
    )(A_x, c, w_mod, A_wq, A_k_cache, A_v_cache, A_wo.T, B_w3, B_w4.T)
```
